```python
import os as _os
_os.environ.setdefault("JAX_PLATFORMS", "cpu")
import jax
import jax.numpy as jnp

def _softmax(x, axis=-1):
    return jax.nn.softmax(x, axis=axis)
def _gelu(x):
    return jax.nn.gelu(x, approximate=True)
def _silu(x):
    return jax.nn.silu(x)
def _sigmoid(x):
    return jax.nn.sigmoid(x)
def _layernorm(x, axis=-1, eps=1e-5):
    m = jnp.mean(x, axis=axis, keepdims=True)
    v = jnp.var(x, axis=axis, keepdims=True)
    return (x - m) / jnp.sqrt(v + eps)
def _scatter_add(tgt, idx, src, axis=0):
    return tgt.at[idx].add(src)
def _segment_sum(src, seg, n):
    return jax.ops.segment_sum(src, seg, n)
class _Rng:
    def __init__(self, key):
        self._k = key
    def _next(self):
        self._k, sub = jax.random.split(self._k)
        return sub
    def normal(self, shape):
        return jax.random.normal(self._next(), shape, dtype=jnp.bfloat16)
    def randint(self, lo, hi, shape):
        return jax.random.randint(self._next(), shape, lo, hi, dtype=jnp.int32)
    def uniform(self, shape, lo=0.0, hi=1.0):
        return jax.random.uniform(self._next(), shape, jnp.bfloat16, lo, hi)
    def permutation(self, n):
        return jax.random.permutation(self._next(), n)


kernel_name = 'sequential_preLN__softmax_full_mha__dense_activation_gelu__prompt'

def setup_inputs():
    _rng = _Rng(jax.random.key(int.from_bytes(__import__("os").urandom(4), "little")))
    _w = (lambda a: (lambda t: t.astype(jnp.bfloat16) if jnp.issubdtype(t.dtype, jnp.floating) else t)(jnp.asarray(a)))
    def _A_setup():
        B, S, D = 1, 2048, 640
        return {
            "x": _w((lambda *s: _rng.normal(s) * 0.05)(B, S, D)),
            "wqkv": _w((lambda *s: _rng.normal(s) * 0.05)(D, 3 * D)),
            "wo": _w((lambda *s: _rng.normal(s) * 0.05)(D, D)),
        }
    _A_in = _A_setup()

    def _B_setup():
        B, S, D, F = 1, 2048, 640, 1536
        return {
            "x": _w((lambda *s: _rng.normal(s) * 0.05)(B, S, D)),
            "w1": _w((lambda *s: _rng.normal(s) * 0.4)(D, F) * (D ** -0.5)),
            "b1": _w((lambda *s: _rng.normal(s) * 0.4)(F) * 0.01),
            "w2": _w((lambda *s: _rng.normal(s) * 0.4)(F, D) * (F ** -0.5)),
            "b2": _w((lambda *s: _rng.normal(s) * 0.05)(D) * 0.01),
        }
    _B_in = _B_setup()

    return {
        "A_x": _A_in["x"],
        "A_wqkv": _A_in["wqkv"],
        "A_wo": _A_in["wo"],
        "B_x": _B_in["x"],
        "B_w1": _B_in["w1"],
        "B_b1": _B_in["b1"],
        "B_w2": _B_in["w2"],
        "B_b2": _B_in["b2"],
    }

def reference(A_x, A_wqkv, A_wo, B_x, B_w1, B_b1, B_w2, B_b2):
    def _A_ref(x, wqkv, wo):
        B, S, D = x.shape
        H = 32; Dh = D // H
        qkv = (lambda x, *d: x.transpose(*d))((x @ wqkv).reshape(B, S, 3, H, Dh), 2, 0, 3, 1, 4)
        q, k, v = qkv[0], qkv[1], qkv[2]
        scale = Dh ** -0.5
        scores = jnp.einsum("bhqd,bhkd->bhqk", q, k) * scale
        p = _softmax(scores, axis=-1)
        o = jnp.einsum("bhqk,bhkd->bhqd", p, v)
        return (lambda x, *d: x.transpose(*d))(o, 0, 2, 1, 3).reshape(B, S, D) @ wo

    def _B_ref(x, w1, b1, w2, b2):
        h = jnp.einsum("bsd,df->bsf", x, w1) + b1
        h = _gelu(h)
        return jnp.einsum("bsf,fd->bsd", h, w2) + b2

    x = A_x
    h = x + _A_ref(_layernorm(x, axis=-1), A_wqkv, A_wo)
    h2 = h + _B_ref(_layernorm(h, axis=-1), B_w1, B_b1, B_w2, B_b2)
    return h2
```

```python
import math

import jax
import jax.numpy as jnp
from jax import lax
import jax.experimental.pallas as pl
import jax.experimental.pallas.tpu as pltpu

_H = 32
_EPS = 1e-5
_TQ = 1024
_TR = 512
_VR = 24
_NT = (((1,), (1,)), ((), ()))
f32, bf16 = jnp.float32, jnp.bfloat16


def _ln(x):
    m = jnp.mean(x, axis=-1, keepdims=True)
    d = x - m
    v = jnp.mean(d * d, axis=-1, keepdims=True)
    return d * lax.rsqrt(v + _EPS)


def _gelu(x):
    c = math.sqrt(2.0 / math.pi)
    return (0.5 * x) * (1.0 + jnp.tanh(x * (c + (c * 0.044715) * (x * x))))


def _kernel(x_hbm, wqkv_hbm, wo_hbm, w1_hbm, b1_ref, w2_hbm, b2_ref, o_hbm,
            wt_ref, qt_ref, k_ref, vt_ref, at_ref,
            wo_ref, w1_ref, w2_ref, o_ref, x_ref, wqkv_ref, sems, isems):
    S, D = x_ref.shape
    Dh = D // _H
    per = 128 // Dh
    nwin = -(-_H // per)
    nchunk = S // _TR
    scale = Dh ** -0.5 * math.log2(math.e)

    loads = [pltpu.make_async_copy(s, d, sems.at[i]) for i, (s, d) in enumerate(
        ((wo_hbm, wo_ref), (w1_hbm, w1_ref), (w2_hbm, w2_ref)))]
    wl = [pltpu.make_async_copy(wqkv_hbm.at[:, j * D:(j + 1) * D],
                                wqkv_ref.at[:, j * D:(j + 1) * D], isems.at[j])
          for j in range(3)]
    xl = [pltpu.make_async_copy(x_hbm.at[r * _TR:(r + 1) * _TR, :],
                                x_ref.at[r * _TR:(r + 1) * _TR, :], isems.at[3 + r])
          for r in range(nchunk)]
    for c in wl + xl:
        c.start()

    for j in range(3):
        wl[j].wait()
        wt_ref[j * D:(j + 1) * D, :] = wqkv_ref[:, j * D:(j + 1) * D].astype(f32).T
    wq = wt_ref[0:D, :].astype(bf16)
    wv = wt_ref[2 * D:3 * D, :].astype(bf16)
    wk = jnp.concatenate(
        [wt_ref[pl.ds(D + min(c * per * Dh, D - 128), 128), :] for c in range(nwin)],
        axis=0).astype(bf16)
    for r in range(nchunk):
        rows = slice(r * _TR, (r + 1) * _TR)
        xl[r].wait()
        if r == nchunk - 1:
            for c in loads:
                c.start()
        xn = _ln(x_ref[rows, :].astype(f32)).astype(bf16)
        kk = lax.dot_general(xn, wk, _NT, preferred_element_type=f32).astype(bf16)
        for c in range(nwin):
            k_ref[c, rows, :] = kk[:, c * 128:(c + 1) * 128]
        qt_ref[:, rows] = lax.dot_general(wq, xn, _NT, preferred_element_type=f32) * scale
        vt_ref[:, rows] = lax.dot_general(wv, xn, _NT, preferred_element_type=f32)
    at_ref[...] = jnp.zeros_like(at_ref)

    def head(h, cols, n, true_max):
        c = h // per
        qs = pl.multiple_of(jnp.minimum(c * per * Dh, D - 128), 8)
        vs = pl.multiple_of((h // 2) * 2 * Dh + (h % 2) * (2 * Dh - _VR), 8)
        rq = lax.broadcasted_iota(jnp.int32, (128, 1), 0) + (qs - h * Dh)
        rv = lax.broadcasted_iota(jnp.int32, (_VR, 1), 0) + (vs - h * Dh)
        own = (rv >= 0) & (rv < Dh)
        q = jnp.where((rq >= 0) & (rq < Dh), qt_ref[pl.ds(qs, 128), cols], 0.0)
        v = jnp.where(own, vt_ref[pl.ds(vs, _VR), :], 1.0).astype(bf16)
        s = jnp.dot(k_ref[c], q.astype(bf16), preferred_element_type=f32)
        if true_max:
            s = s - jnp.max(s, axis=0, keepdims=True)
        o = jnp.dot(v, jnp.exp2(s).astype(bf16), preferred_element_type=f32)
        l = jnp.where(h % 2 == 0, o[_VR - 1:_VR, :], o[0:1, :])
        dst = (pl.ds(vs, _VR), cols)
        at_ref[dst] = jnp.where(own, o * (1.0 / l), at_ref[dst])
        safe = (l > 2.0 ** -40) & (l < 2.0 ** 60) & (jnp.abs(o) < 2.0 ** 120)
        return jnp.where(safe, 0.0, 1.0)

    def fast(h, bad):
        for j in range(S // _TQ):
            bad = jnp.maximum(bad, head(h, slice(j * _TQ, (j + 1) * _TQ), _TQ, False))
        return bad

    bad = lax.fori_loop(0, _H, fast, jnp.zeros((_VR, _TQ), f32))

    @pl.when(jnp.max(bad) > 0.0)
    def _():
        nq = S // 256

        def exact(i, carry):
            head(i // nq, pl.ds(pl.multiple_of((i % nq) * 256, 256), 256), 256, True)
            return carry
        lax.fori_loop(0, _H * nq, exact, 0)

    for c in loads:
        c.wait()
    stores = []
    for r in range(nchunk):
        rows = slice(r * _TR, (r + 1) * _TR)
        a = at_ref[:, rows].T.astype(bf16)
        h1 = x_ref[rows, :].astype(f32) + jnp.dot(a, wo_ref[...], preferred_element_type=f32)
        u = jnp.dot(_ln(h1).astype(bf16), w1_ref[...], preferred_element_type=f32)
        g = _gelu(u + b1_ref[...].astype(f32).reshape(1, -1)).astype(bf16)
        y = jnp.dot(g, w2_ref[...], preferred_element_type=f32)
        o_ref[rows, :] = (h1 + y + b2_ref[...].astype(f32).reshape(1, -1)).astype(o_ref.dtype)
        st = pltpu.make_async_copy(o_ref.at[rows, :], o_hbm.at[rows, :], sems.at[3 + r])
        st.start()
        stores.append(st)
    for st in stores:
        st.wait()


@jax.jit
def pallas_sequential_preLN__softmax_full_mha__dense_activation_gelu__prompt_kernel(
    A_x: jax.Array,
    A_wqkv: jax.Array,
    A_wo: jax.Array,
    B_x: jax.Array,
    B_w1: jax.Array,
    B_b1: jax.Array,
    B_w2: jax.Array,
    B_b2: jax.Array,
):
    del B_x
    B, S, D = A_x.shape
    assert B == 1 and D == 20 * _H
    nwin = -(-_H // (128 // (D // _H)))
    vm = pl.BlockSpec(memory_space=pltpu.VMEM)
    hbm = pl.BlockSpec(memory_space=pl.ANY)
    out = pl.pallas_call(
        _kernel,
        out_shape=jax.ShapeDtypeStruct((S, D), A_x.dtype),
        in_specs=[hbm, hbm, hbm, hbm, vm, hbm, vm],
        out_specs=hbm,
        scratch_shapes=[
            pltpu.VMEM((3 * D, D), f32),
            pltpu.VMEM((D, S), f32),
            pltpu.VMEM((nwin, S, 128), bf16),
            pltpu.VMEM((D, S), f32),
            pltpu.VMEM((D, S), f32),
            pltpu.VMEM(A_wo.shape, A_wo.dtype),
            pltpu.VMEM(B_w1.shape, B_w1.dtype),
            pltpu.VMEM(B_w2.shape, B_w2.dtype),
            pltpu.VMEM((S, D), A_x.dtype),
            pltpu.VMEM((S, D), A_x.dtype),
            pltpu.VMEM(A_wqkv.shape, A_wqkv.dtype),
            pltpu.SemaphoreType.DMA((3 + S // _TR,)),
            pltpu.SemaphoreType.DMA((3 + S // _TR,)),
        ],
        compiler_params=pltpu.CompilerParams(vmem_limit_bytes=110 * 1024 * 1024),
    )(A_x.reshape(S, D), A_wqkv, A_wo, B_w1, B_b1, B_w2, B_b2)
    return out.reshape(B, S, D)
```
